```python
import jax
import jax.numpy as jnp

def _softmax(x, axis=-1):
    return jax.nn.softmax(x, axis=axis)
def _gelu(x):
    return jax.nn.gelu(x, approximate=True)
def _silu(x):
    return jax.nn.silu(x)
def _sigmoid(x):
    return jax.nn.sigmoid(x)
def _layernorm(x, axis=-1, eps=1e-5):
    m = jnp.mean(x, axis=axis, keepdims=True)
    v = jnp.var(x, axis=axis, keepdims=True)
    return (x - m) / jnp.sqrt(v + eps)
def _scatter_add(tgt, idx, src, axis=0):
    return tgt.at[idx].add(src)
def _segment_sum(src, seg, n):
    return jax.ops.segment_sum(src, seg, n)
class _Rng:
    def __init__(self, key):
        self._k = key
    def _next(self):
        self._k, sub = jax.random.split(self._k)
        return sub
    def normal(self, shape):
        return jax.random.normal(self._next(), shape, dtype=jnp.bfloat16)
    def randint(self, lo, hi, shape):
        return jax.random.randint(self._next(), shape, lo, hi, dtype=jnp.int32)
    def uniform(self, shape, lo=0.0, hi=1.0):
        return jax.random.uniform(self._next(), shape, jnp.bfloat16, lo, hi)
    def permutation(self, n):
        return jax.random.permutation(self._next(), n)


kernel_name = 'standalone__standard_2d_1d_3d_conv__vision'

def setup_inputs():
    _rng = _Rng(jax.random.key(int.from_bytes(__import__("os").urandom(4), "little")))
    _w = (lambda a: (lambda t: t.astype(jnp.bfloat16) if jnp.issubdtype(t.dtype, jnp.floating) else t)(jnp.asarray(a)))
    H = W = 384
    C = 384
    K = 1
    return {
        "x": _w((lambda *s: _rng.normal(s) * 0.05)(1, H, W, C)),
        "w": _w((lambda *s: _rng.normal(s) * 0.05)(K, K, C, C)),
        "b": _w((lambda *s: _rng.normal(s) * 0.05)(C)),
    }

def reference(x, w, b):
    B, H, W, Cin = x.shape
    K = w.shape[0]
    pl = (K - 1) // 2
    pr = K // 2
    xp = jnp.pad(x, ((0, 0), (pl, pr), (pl, pr), (0, 0)))
    out = sum(
        jnp.einsum('bhwc,cd->bhwd', xp[:, i:i+H, j:j+W, :], w[i, j])
        for i in range(K) for j in range(K)
    )
    return out + b[None, None, None, :]
```

```python
import jax
import jax.numpy as jnp
from jax import lax
import jax.experimental.pallas as pl
import jax.experimental.pallas.tpu as pltpu

_S = 6
_DIST = 2048
_RC = 128
_RR = 8
_RW = 16
_P = 6
_W0 = 9
_CB = 2
_KW = (3, 4)
_NW = 16


def _make_kernel(n_super, cin, cout):
    cpa = _DIST // _RC
    nch = n_super * cpa
    nu = nch // 2
    t1 = nu - _P
    assert n_super % 2 == 0 and (nch - t1) % _CB == 0
    n2 = (nch - t1) // _CB

    def kernel(x_hbm, w_hbm, b_hbm, o_hbm, buf, w_v, b_v, b_f32, rsem, wsem, csem):
        def rd_issue(u):
            m = u // cpa
            i = u % cpa
            r0 = pl.multiple_of(i * _RC, _RC)
            for k in range(_RC // _RR):
                for h in (1, 0):
                    a = 2 * m + h
                    pltpu.make_async_copy(
                        x_hbm.at[a, :, pl.ds(r0 + k * _RR, _RR), :],
                        buf.at[a * cpa + i, :, pl.ds(k * _RR, _RR), :],
                        rsem.at[u % _P],
                    ).start(priority=h)

        def rd_wait(u):
            two = buf.at[pl.ds(0, 2)]
            pltpu.make_async_copy(two, two, rsem.at[u % _P]).wait()

        def wr_issue(c):
            a = c // cpa
            i = c % cpa
            r0 = pl.multiple_of(i * _RC, _RC)
            for k in range(_RC // _RW):
                pltpu.make_async_copy(
                    buf.at[c, :, pl.ds(k * _RW, _RW), :],
                    o_hbm.at[a, :, pl.ds(r0 + k * _RW, _RW), :],
                    wsem.at[c % _NW],
                ).start()

        def wr_wait(c):
            one = buf.at[0]
            pltpu.make_async_copy(one, one, wsem.at[c % _NW]).wait()

        def compute(c, n):
            x = buf[pl.ds(c, n)].reshape(n * _S * _RC, cin)
            acc = jnp.dot(x, w_v[...], preferred_element_type=jnp.float32)
            y = (acc + b_f32[...]).astype(buf.dtype)
            buf[pl.ds(c, n)] = y.reshape(n, _S, _RC, cout)

        w_cp = pltpu.make_async_copy(w_hbm, w_v, csem.at[0])
        b_cp = pltpu.make_async_copy(b_hbm, b_v, csem.at[1])
        rd_issue(0)
        w_cp.start()
        b_cp.start()

        def prologue(u, carry):
            rd_issue(u)
            return carry

        lax.fori_loop(1, _P, prologue, 0)
        w_cp.wait()
        b_cp.wait()
        b_f32[...] = b_v[...].astype(jnp.float32).reshape(1, cout)

        def phase1(t, carry):
            rd_wait(t)
            rd_issue(t + _P)
            compute(t, 1)
            return carry

        lax.fori_loop(0, t1, phase1, 0)

        def first_writes(c, carry):
            wr_issue(c)
            return carry

        lax.fori_loop(0, _W0, first_writes, 0)

        def next_write(c, carry):
            @pl.when(c >= _NW)
            def _():
                wr_wait(c - _NW)

            wr_issue(c)
            return carry

        def phase2(s, wn):
            c = t1 + s * _CB
            compute(c, _CB)

            @pl.when(s == 0)
            def _():
                for u in range(t1, nu):
                    rd_wait(u)

            kw = jnp.where(s % 2 == 0, _KW[0], _KW[1])
            hi = jnp.minimum(wn + kw, c + _CB)
            lax.fori_loop(wn, hi, next_write, 0)
            return hi

        wn = lax.fori_loop(0, n2, phase2, _W0)
        lax.fori_loop(wn, nch, next_write, 0)
        for c in range(nch - _NW, nch):
            wr_wait(c)

    return kernel, nch


@jax.jit
def pallas_standalone__standard_2d_1d_3d_conv__vision_kernel(
    x: jax.Array,
    w: jax.Array,
    b: jax.Array,
):
    B, H, W, cin = x.shape
    kh, kw, _, cout = w.shape
    assert kh == 1 and kw == 1 and cin == cout
    m = B * H * W
    n_super = m // (_S * _DIST)
    assert n_super * _S * _DIST == m
    kernel, nch = _make_kernel(n_super, cin, cout)
    out = pl.pallas_call(
        kernel,
        in_specs=[pl.BlockSpec(memory_space=pl.ANY)] * 3,
        out_specs=pl.BlockSpec(memory_space=pl.ANY),
        out_shape=jax.ShapeDtypeStruct((n_super, _S, _DIST, cout), x.dtype),
        scratch_shapes=[
            pltpu.VMEM((nch, _S, _RC, cin), x.dtype),
            pltpu.VMEM((cin, cout), w.dtype),
            pltpu.VMEM((cout,), b.dtype),
            pltpu.VMEM((1, cout), jnp.float32),
            pltpu.SemaphoreType.DMA((_P,)),
            pltpu.SemaphoreType.DMA((_NW,)),
            pltpu.SemaphoreType.DMA((2,)),
        ],
        compiler_params=pltpu.CompilerParams(
            vmem_limit_bytes=120 * 1024 * 1024,
            disable_bounds_checks=True,
            disable_semaphore_checks=True,
        ),
    )(x.reshape(n_super, _S, _DIST, cin), w.reshape(cin, cout), b)
    return out.reshape(B, H, W, cout)
```

```python
import jax
import jax.numpy as jnp
from jax import lax
import jax.experimental.pallas as pl
import jax.experimental.pallas.tpu as pltpu

_S = 6
_DIST = 2048
_RC = 128
_RR = 8
_RW = 16
_P = 6
_TL = 13
_W0 = 9
_CB = 2
_KW = (3, 4)
_NW = 16


def _make_kernel(n_super, cin, cout):
    cpa = _DIST // _RC
    nch = n_super * cpa
    nu = nch // 2
    kr = _RC // _RR
    t1 = nu - _P
    assert n_super % 2 == 0 and (nch - t1) % _CB == 0 and 0 < _TL < kr and _W0 <= min(t1, _NW)
    n2 = (nch - t1) // _CB

    def row0(i):
        return i * _RC if isinstance(i, int) else pl.multiple_of(i * _RC, _RC)

    def kernel(x_hbm, w_hbm, b_hbm, o_hbm, buf, w_v, b_v, b_f32, rsem, wsem, csem):
        def rd_copy(u, h, k0, nk, sem=None):
            i = u % cpa
            a = 2 * (u // cpa) + h
            return pltpu.make_async_copy(
                x_hbm.at[a, :, pl.ds(row0(i) + k0 * _RR, nk * _RR), :],
                buf.at[a * cpa + i, :, pl.ds(k0 * _RR, nk * _RR), :],
                rsem.at[2 * (u % _P) + h] if sem is None else sem,
            )

        def rd_issue(u):
            for k in range(kr):
                for h in (1, 0):
                    rd_copy(u, h, k, 1).start(priority=h)

        def rd_wait(u):
            rd_copy(u, 0, 0, kr).wait()
            rd_copy(u, 1, 0, kr).wait()

        def wr_copy(c, r, n):
            return pltpu.make_async_copy(
                buf.at[c, :, pl.ds(r, n), :],
                o_hbm.at[c // cpa, :, pl.ds(row0(c % cpa) + r, n), :],
                wsem.at[c % _NW],
            )

        def wr_issue(c):
            for k in range(_RC // _RW):
                wr_copy(c, k * _RW, _RW).start()

        def wr_wait(c):
            wr_copy(c, 0, _RC).wait()

        def compute(c, n):
            x = buf[pl.ds(c, n)].reshape(n * _S * _RC, cin)
            acc = jnp.dot(x, w_v[...], preferred_element_type=jnp.float32)
            y = (acc + b_f32[...]).astype(buf.dtype)
            buf[pl.ds(c, n)] = y.reshape(n, _S, _RC, cout)

        w_cp = pltpu.make_async_copy(w_hbm, w_v, csem.at[0])
        b_cp = pltpu.make_async_copy(b_hbm, b_v, csem.at[1])
        rd_issue(0)
        w_cp.start()
        b_cp.start()

        def prologue(u, carry):
            rd_issue(u)
            return carry

        lax.fori_loop(1, _P, prologue, 0)
        w_cp.wait()
        b_cp.wait()
        b_f32[...] = b_v[...].astype(jnp.float32).reshape(1, cout)

        def phase1(t, carry):
            rd_wait(t)
            rd_issue(t + _P)
            compute(t, 1)
            return carry

        lax.fori_loop(0, t1 - 1, phase1, 0)

        rd_wait(t1 - 1)
        for k in range(kr):
            rd_copy(nu - 1, 1, k, 1, csem.at[2] if k >= kr - _TL else None).start(priority=1)
            rd_copy(nu - 1, 0, k, 1).start(priority=0)
        compute(t1 - 1, 1)
        for u in range(t1, nu - 1):
            rd_wait(u)
        rd_copy(nu - 1, 0, 0, kr).wait()
        rd_copy(nu - 1, 1, 0, kr - _TL).wait()

        def first_writes(c, carry):
            wr_issue(c)
            return carry

        lax.fori_loop(0, _W0, first_writes, 0)
        rd_copy(nu - 1, 1, kr - _TL, _TL, csem.at[2]).wait()

        def next_write(c, carry):
            @pl.when(c >= _NW)
            def _():
                wr_wait(c - _NW)

            wr_issue(c)
            return carry

        def phase2(s, wn):
            c = t1 + s * _CB
            compute(c, _CB)
            kw = jnp.where(s % 2 == 0, _KW[0], _KW[1])
            hi = jnp.minimum(wn + kw, c + _CB)
            lax.fori_loop(wn, hi, next_write, 0)
            return hi

        wn = lax.fori_loop(0, n2, phase2, _W0)
        lax.fori_loop(wn, nch, next_write, 0)
        for c in range(nch - _NW, nch):
            wr_wait(c)

    return kernel, nch


@jax.jit
def pallas_standalone__standard_2d_1d_3d_conv__vision_kernel(
    x: jax.Array,
    w: jax.Array,
    b: jax.Array,
):
    B, H, W, cin = x.shape
    kh, kw, _, cout = w.shape
    assert kh == 1 and kw == 1 and cin == cout
    m = B * H * W
    n_super = m // (_S * _DIST)
    assert n_super * _S * _DIST == m
    kernel, nch = _make_kernel(n_super, cin, cout)
    out = pl.pallas_call(
        kernel,
        in_specs=[pl.BlockSpec(memory_space=pl.ANY)] * 3,
        out_specs=pl.BlockSpec(memory_space=pl.ANY),
        out_shape=jax.ShapeDtypeStruct((n_super, _S, _DIST, cout), x.dtype),
        scratch_shapes=[
            pltpu.VMEM((nch, _S, _RC, cin), x.dtype),
            pltpu.VMEM((cin, cout), w.dtype),
            pltpu.VMEM((cout,), b.dtype),
            pltpu.VMEM((1, cout), jnp.float32),
            pltpu.SemaphoreType.DMA((2 * _P,)),
            pltpu.SemaphoreType.DMA((_NW,)),
            pltpu.SemaphoreType.DMA((3,)),
        ],
        compiler_params=pltpu.CompilerParams(
            vmem_limit_bytes=120 * 1024 * 1024,
            disable_bounds_checks=True,
            disable_semaphore_checks=True,
        ),
    )(x.reshape(n_super, _S, _DIST, cin), w.reshape(cin, cout), b)
    return out.reshape(B, H, W, cout)
```

```python
import jax
import jax.numpy as jnp
from jax import lax
import jax.experimental.pallas as pl
import jax.experimental.pallas.tpu as pltpu

_S = 6
_DIST = 2048
_RC = 128
_RR = 8
_RW = 16
_P = 6
_TL = 13
_W0 = 9
_CB = 2
_KW = (3, 4)
_NW = 16


def _make_kernel(n_super, cin, cout):
    cpa = _DIST // _RC
    nch = n_super * cpa
    nu = nch // 2
    kr = _RC // _RR
    t1 = nu - _P
    assert n_super % 2 == 0 and (nch - t1) % _CB == 0 and 0 < _TL < kr and _W0 <= min(t1, _NW)
    n2 = (nch - t1) // _CB

    def row0(i):
        return i * _RC if isinstance(i, int) else pl.multiple_of(i * _RC, _RC)

    def kernel(x_hbm, w_hbm, b_hbm, o_hbm, buf, w_v, b_v, b_f32, rsem, wsem, csem):
        def rd_copy(u, h, k0, nk, sem=None):
            i = u % cpa
            a = 2 * (u // cpa) + h
            return pltpu.make_async_copy(
                x_hbm.at[a, :, pl.ds(row0(i) + k0 * _RR, nk * _RR), :],
                buf.at[a * cpa + i, :, pl.ds(k0 * _RR, nk * _RR), :],
                rsem.at[2 * (u % _P) + h] if sem is None else sem,
            )

        def rd_issue(u):
            for k in range(kr):
                for h in (1, 0):
                    rd_copy(u, h, k, 1).start(priority=h)

        def rd_wait(u):
            rd_copy(u, 0, 0, kr).wait()
            rd_copy(u, 1, 0, kr).wait()

        def wr_copy(c, r, n):
            return pltpu.make_async_copy(
                buf.at[c, :, pl.ds(r, n), :],
                o_hbm.at[c // cpa, :, pl.ds(row0(c % cpa) + r, n), :],
                wsem.at[c % _NW],
            )

        def wr_issue(c):
            for k in range(_RC // _RW):
                wr_copy(c, k * _RW, _RW).start()

        def wr_wait(c):
            wr_copy(c, 0, _RC).wait()

        def compute(c, n):
            x = buf[pl.ds(c, n)].reshape(n * _S * _RC, cin)
            acc = jnp.dot(x, w_v[...], preferred_element_type=jnp.float32)
            y = (acc + b_f32[...]).astype(buf.dtype)
            buf[pl.ds(c, n)] = y.reshape(n, _S, _RC, cout)

        w_cp = pltpu.make_async_copy(w_hbm, w_v, csem.at[0])
        b_cp = pltpu.make_async_copy(b_hbm, b_v, csem.at[1])
        rd_issue(0)
        w_cp.start()
        b_cp.start()

        def prologue(u, carry):
            rd_issue(u)
            return carry

        lax.fori_loop(1, _P, prologue, 0)
        w_cp.wait()
        b_cp.wait()
        b_f32[...] = b_v[...].astype(jnp.float32).reshape(1, cout)

        def phase1(t, carry):
            rd_wait(t)
            rd_issue(t + _P)
            compute(t, 1)
            return carry

        lax.fori_loop(0, t1 - 1, phase1, 0)

        rd_wait(t1 - 1)
        for k in range(kr):
            rd_copy(nu - 1, 1, k, 1, csem.at[2] if k >= kr - _TL else None).start(priority=1)
            rd_copy(nu - 1, 0, k, 1).start(priority=0)
        compute(t1 - 1, 1)
        for u in range(t1, nu - 1):
            rd_wait(u)
        rd_copy(nu - 1, 0, 0, kr).wait()
        rd_copy(nu - 1, 1, 0, kr - _TL).wait()

        def first_writes(c, carry):
            wr_issue(c)
            return carry

        lax.fori_loop(0, _W0, first_writes, 0)
        rd_copy(nu - 1, 1, kr - _TL, _TL, csem.at[2]).wait()

        def next_write(c, carry):
            @pl.when(c >= _NW)
            def _():
                wr_wait(c - _NW)

            wr_issue(c)
            return carry

        def phase2(s, wn):
            c = t1 + s * _CB
            compute(c, _CB)
            kw = jnp.where(s % 2 == 0, _KW[0], _KW[1])
            hi = jnp.minimum(wn + kw, c + _CB)
            lax.fori_loop(wn, hi, next_write, 0)
            return hi

        wn = lax.fori_loop(0, n2, phase2, _W0)
        lax.fori_loop(wn, nch, next_write, 0)
        for c in range(nch - _NW, nch):
            wr_wait(c)

    return kernel, nch


def _compiler_params():
    kwargs = dict(vmem_limit_bytes=120 * 1024 * 1024, disable_bounds_checks=True)
    try:
        return pltpu.CompilerParams(disable_semaphore_checks=True, **kwargs)
    except TypeError:
        return pltpu.CompilerParams(**kwargs)


@jax.jit
def pallas_standalone__standard_2d_1d_3d_conv__vision_kernel(
    x: jax.Array,
    w: jax.Array,
    b: jax.Array,
):
    B, H, W, cin = x.shape
    kh, kw, _, cout = w.shape
    assert kh == 1 and kw == 1 and cin == cout
    m = B * H * W
    n_super = m // (_S * _DIST)
    assert n_super * _S * _DIST == m
    kernel, nch = _make_kernel(n_super, cin, cout)
    out = pl.pallas_call(
        kernel,
        in_specs=[pl.BlockSpec(memory_space=pl.ANY)] * 3,
        out_specs=pl.BlockSpec(memory_space=pl.ANY),
        out_shape=jax.ShapeDtypeStruct((n_super, _S, _DIST, cout), x.dtype),
        scratch_shapes=[
            pltpu.VMEM((nch, _S, _RC, cin), x.dtype),
            pltpu.VMEM((cin, cout), w.dtype),
            pltpu.VMEM((cout,), b.dtype),
            pltpu.VMEM((1, cout), jnp.float32),
            pltpu.SemaphoreType.DMA((2 * _P,)),
            pltpu.SemaphoreType.DMA((_NW,)),
            pltpu.SemaphoreType.DMA((3,)),
        ],
        compiler_params=_compiler_params(),
    )(x.reshape(n_super, _S, _DIST, cin), w.reshape(cin, cout), b)
    return out.reshape(B, H, W, cout)
```

```python
import jax
import jax.numpy as jnp
from jax import lax
import jax.experimental.pallas as pl
import jax.experimental.pallas.tpu as pltpu

_TPB = 512
_RT = 170
_S = 6
_Q = 17
_P = 5
_NR = 8
_SK = 26
_TL = 12
_PW = 6
_WT = 30
_W0 = 14
_KB = 6
_NW = 32


def _when(cond, fn):
    if isinstance(cond, bool):
        if cond:
            fn()
    else:
        pl.when(cond)(fn)


def _make_kernel(nb, c):
    cpg = _RT // _Q
    ng = nb // _S
    nu = ng // 2 * cpg
    nch = ng * cpg
    sk1 = _SK - _Q
    t1 = nu - 1 - _P
    n2 = (nch - t1) // 2
    upg = (_TPB - 2) // _WT
    nwu = ng * upg
    ct = _W0 + _KB * n2
    assert c == 3 * 128 and ng * _S == nb and ng % 2 == 0 and _S % 3 == 0 and cpg % 2 == 0
    assert 0 < sk1 < _Q and _P + 2 <= _NR and 0 < _TL < _Q and t1 % 2 == 0 and t1 >= 2 * cpg
    assert upg * _WT == _TPB - 2 and _WT % _PW == 0 and _KB <= upg
    assert _W0 <= min(_NW, 2 * upg) and _NW <= ct <= nwu
    for s in range(n2):
        cc = t1 + 2 * s
        assert _W0 + _KB * (s + 1) <= (cc // cpg) * upg + (3 * _Q * (cc % cpg)) // _WT

    def kernel(x_hbm, w_hbm, b_hbm, o_hbm, buf, w_v, b_v, b_f32, rsem, hsem, wsem, tsem, csem):
        def rd_copy(u, h, k0, nk, sem=None):
            blocks = pl.ds((2 * (u // cpg) + h) * _S, _S)
            tiles = pl.ds(2 + 3 * (_Q * (u % cpg) + k0), 3 * nk)
            return pltpu.make_async_copy(
                x_hbm.at[blocks, tiles], buf.at[blocks, tiles],
                rsem.at[2 * (u % _NR) + h] if sem is None else sem)

        def rd_head(m, h):
            blocks = pl.ds((2 * m + h) * _S, _S)
            return pltpu.make_async_copy(
                x_hbm.at[blocks, pl.ds(0, 2)], buf.at[blocks, pl.ds(0, 2)], hsem.at[h])

        def rd_step(u, n=_Q):
            for k in range(n):
                if k < _Q - sk1:
                    rd_copy(u + 1, 1, sk1 + k, 1).start(priority=1)
                else:
                    if k == _Q - sk1:
                        _when((u + 2) % cpg == 0,
                              lambda: rd_head((u + 2) // cpg, 1).start(priority=1))
                    rd_copy(u + 2, 1, k - (_Q - sk1), 1).start(priority=1)
                if k == 0:
                    _when(u % cpg == 0, lambda: rd_head(u // cpg, 0).start(priority=0))
                rd_copy(u, 0, k, 1).start(priority=0)

        def rd_wait(u):
            def heads():
                rd_head(u // cpg, 0).wait()
                rd_head(u // cpg, 1).wait()

            _when(u % cpg == 0, heads)
            rd_copy(u, 0, 0, _Q).wait()
            rd_copy(u, 1, 0, _Q).wait()

        def wr_copy(v, g, i, t0, nt):
            blocks, tiles = pl.ds(g * _S, _S), pl.ds(i * _WT + t0, nt)
            return pltpu.make_async_copy(
                buf.at[blocks, tiles], o_hbm.at[blocks, tiles], wsem.at[v % _NW])

        def wr_tail(g):
            blocks, tiles = pl.ds(g * _S, _S), pl.ds(_TPB - 2, 2)
            return pltpu.make_async_copy(
                buf.at[blocks, tiles], o_hbm.at[blocks, tiles], tsem.at[g])

        def wr_issue(v, g, i):
            for k in range(_WT // _PW):
                wr_copy(v, g, i, k * _PW, _PW).start()
            _when(i == upg - 1, lambda: wr_tail(g).start())

        def wr_wait(v):
            wr_copy(v, v // upg, v % upg, 0, _WT).wait()

        def linear(x):
            acc = jnp.dot(x, w_v[...], preferred_element_type=jnp.float32)
            return (acc + b_f32[...]).astype(buf.dtype)

        def compute(cc, n):
            b0, q0, nq = (cc // cpg) * _S, (cc % cpg) * _Q, n * _Q
            tiles = [pl.ds(j % 3 + 3 * q0, 3 * nq) for j in range(_S)]
            xs = []
            for j in range(_S):
                x3 = buf[b0 + j, tiles[j]].reshape(nq, 3, 8, 128)
                xs.append(jnp.concatenate(
                    [x3[:, k].reshape(nq * 8, 128) for k in range(3)], axis=1))
            y = linear(jnp.concatenate(xs, axis=0))
            for j in range(_S):
                yj = y[j * nq * 8:(j + 1) * nq * 8]
                cols = [yj[:, k * 128:(k + 1) * 128].reshape(nq, 1, 8, 128) for k in range(3)]
                buf[b0 + j, tiles[j]] = jnp.concatenate(cols, axis=1).reshape(3 * nq, 8, 128)

        def compute_straddlers(b_lo, b_hi):
            rows = []
            for b in range(b_lo, b_hi, 3):
                rows.append([(b, _TPB - 2), (b, _TPB - 1), (b + 1, 0)])
                rows.append([(b + 1, _TPB - 1), (b + 2, 0), (b + 2, 1)])
            y = linear(jnp.concatenate(
                [jnp.concatenate([buf[b, t] for b, t in row], axis=1) for row in rows], axis=0))
            for i, row in enumerate(rows):
                for k, (b, t) in enumerate(row):
                    buf[b, t] = y[8 * i:8 * (i + 1), 128 * k:128 * (k + 1)]

        w_cp = pltpu.make_async_copy(w_hbm, w_v, csem.at[0])
        b_cp = pltpu.make_async_copy(b_hbm, b_v, csem.at[1])
        rd_head(0, 1).start(priority=1)
        for k in range(_SK):
            rd_copy(k // _Q, 1, k % _Q, 1).start(priority=1)
        rd_step(0)
        w_cp.start()
        b_cp.start()

        def prologue(u, carry):
            rd_step(u)
            return carry

        lax.fori_loop(1, _P, prologue, 0)
        w_cp.wait()
        b_cp.wait()
        b_f32[...] = b_v[...].astype(jnp.float32).reshape(1, c)

        def phase1(t, carry):
            rd_wait(t)
            rd_step(t + _P)
            compute(t, 1)
            return carry

        lax.fori_loop(0, t1 - 1, phase1, 0)

        rd_wait(t1 - 1)
        rd_step(nu - 2, _Q - sk1)
        rest = [(nu - 2, k) for k in range(_Q - sk1, _Q)] + [(nu - 1, k) for k in range(_Q)]
        early, late = rest[:_SK - _TL], rest[_SK - _TL:]
        for j in range(max(len(early), len(late))):
            if j < len(late):
                rd_copy(late[j][0], 0, late[j][1], 1, csem.at[2]).start(priority=1)
            if j < len(early):
                rd_copy(early[j][0], 0, early[j][1], 1).start(priority=0)
        compute(t1 - 1, 1)
        compute_straddlers(0, 2 * _S)
        for u in range(t1, nu - 1):
            rd_wait(u)
        rd_copy(nu - 1, 1, 0, _Q).wait()
        rd_copy(nu - 1, 0, 0, _Q - _TL).wait()
        for v in range(_W0):
            wr_issue(v, v // upg, v % upg)
        rd_copy(nu - 1, 0, _Q - _TL, _TL, csem.at[2]).wait()
        compute_straddlers(2 * _S, nb)

        def phase2(s, carry):
            v0 = _W0 + _KB * s
            g0, i0 = v0 // upg, v0 % upg
            for k in range(_KB):
                _when(v0 + k >= _NW, lambda: wr_wait(v0 + k - _NW))
                wrap = jnp.where(i0 + k >= upg, 1, 0)
                wr_issue(v0 + k, g0 + wrap, i0 + k - upg * wrap)
            compute(t1 + 2 * s, 2)
            return carry

        lax.fori_loop(0, n2, phase2, 0)
        for v in range(ct, nwu):
            wr_wait(v - _NW)
            wr_issue(v, v // upg, v % upg)
        for g in range(ng - 1):
            wr_tail(g).wait()
        for v in range(nwu - _NW, nwu):
            wr_wait(v)
        wr_tail(ng - 1).wait()

    return kernel, ng


def _compiler_params():
    kwargs = dict(vmem_limit_bytes=120 * 1024 * 1024, disable_bounds_checks=True)
    try:
        return pltpu.CompilerParams(disable_semaphore_checks=True, **kwargs)
    except TypeError:
        return pltpu.CompilerParams(**kwargs)


@jax.jit
def pallas_standalone__standard_2d_1d_3d_conv__vision_kernel(
    x: jax.Array,
    w: jax.Array,
    b: jax.Array,
):
    B, H, W, c = x.shape
    assert w.shape == (1, 1, c, c) and b.shape == (c,)
    m = B * H * W
    nb = m // 8 * 3 // _TPB
    assert nb * _TPB * 8 == m * 3
    kernel, ng = _make_kernel(nb, c)
    tiled = (nb, _TPB, 8, 128)
    x_tiles = x.reshape(m // 8, 8, 3, 128).transpose(0, 2, 1, 3).reshape(tiled)
    out = pl.pallas_call(
        kernel,
        in_specs=[pl.BlockSpec(memory_space=pl.ANY)] * 3,
        out_specs=pl.BlockSpec(memory_space=pl.ANY),
        out_shape=jax.ShapeDtypeStruct(tiled, x.dtype),
        scratch_shapes=[
            pltpu.VMEM(tiled, x.dtype),
            pltpu.VMEM((c, c), w.dtype),
            pltpu.VMEM((c,), b.dtype),
            pltpu.VMEM((1, c), jnp.float32),
            pltpu.SemaphoreType.DMA((2 * _NR,)),
            pltpu.SemaphoreType.DMA((2,)),
            pltpu.SemaphoreType.DMA((_NW,)),
            pltpu.SemaphoreType.DMA((ng,)),
            pltpu.SemaphoreType.DMA((3,)),
        ],
        compiler_params=_compiler_params(),
    )(x_tiles, w.reshape(c, c), b)
    return out.reshape(m // 8, 3, 8, 128).transpose(0, 2, 1, 3).reshape(B, H, W, c)
```
